```python
import os as _os
_os.environ.setdefault("JAX_PLATFORMS", "cpu")
import jax
import jax.numpy as jnp

def _softmax(x, axis=-1):
    return jax.nn.softmax(x, axis=axis)
def _gelu(x):
    return jax.nn.gelu(x, approximate=True)
def _silu(x):
    return jax.nn.silu(x)
def _sigmoid(x):
    return jax.nn.sigmoid(x)
def _layernorm(x, axis=-1, eps=1e-5):
    m = jnp.mean(x, axis=axis, keepdims=True)
    v = jnp.var(x, axis=axis, keepdims=True)
    return (x - m) / jnp.sqrt(v + eps)
def _scatter_add(tgt, idx, src, axis=0):
    return tgt.at[idx].add(src)
def _segment_sum(src, seg, n):
    return jax.ops.segment_sum(src, seg, n)
class _Rng:
    def __init__(self, key):
        self._k = key
    def _next(self):
        self._k, sub = jax.random.split(self._k)
        return sub
    def normal(self, shape):
        return jax.random.normal(self._next(), shape, dtype=jnp.bfloat16)
    def randint(self, lo, hi, shape):
        return jax.random.randint(self._next(), shape, lo, hi, dtype=jnp.int32)
    def uniform(self, shape, lo=0.0, hi=1.0):
        return jax.random.uniform(self._next(), shape, jnp.bfloat16, lo, hi)
    def permutation(self, n):
        return jax.random.permutation(self._next(), n)


kernel_name = 'interleave_layers__mha_block__dense_activation_mish__prompt'

def setup_inputs():
    _rng = _Rng(jax.random.key(int.from_bytes(__import__("os").urandom(4), "little")))
    _w = (lambda a: (lambda t: t.astype(jnp.bfloat16) if jnp.issubdtype(t.dtype, jnp.floating) else t)(jnp.asarray(a)))
    def _A_setup():
        B, S, D, H = 1, 2048, 512, 32
        return {
            "x": _w((lambda *s: _rng.normal(s) * 0.05)(B, S, D)),
            "wqkv": _w((lambda *s: _rng.normal(s) * 0.05)(D, 3 * D)),
            "wo": _w((lambda *s: _rng.normal(s) * 0.05)(D, D)),
        }
    _A_in = _A_setup()

    def _B_setup():
        B, S, D, F = 1, 2048, 512, 1792
        return {
            "x": _w((lambda *s: _rng.normal(s) * 0.05)(B, S, D)),
            "w1": _w((lambda *s: _rng.normal(s) * 0.4)(D, F) * (D ** -0.5)),
            "b1": _w((lambda *s: _rng.normal(s) * 0.4)(F)),
            "w2": _w((lambda *s: _rng.normal(s) * 0.4)(F, D) * (F ** -0.5)),
        }
    _B_in = _B_setup()

    return {
        "A_x": _A_in["x"],
        "A_wqkv": _A_in["wqkv"],
        "A_wo": _A_in["wo"],
        "B_x": _B_in["x"],
        "B_w1": _B_in["w1"],
        "B_b1": _B_in["b1"],
        "B_w2": _B_in["w2"],
    }

def reference(A_x, A_wqkv, A_wo, B_x, B_w1, B_b1, B_w2):
    def _A_ref(x, wqkv, wo):
        B, S, D = x.shape
        H = 32
        Dh = D // H
        qkv = (lambda x, *d: x.transpose(*d))((x @ wqkv).reshape(B, S, 3, H, Dh), 2, 0, 3, 1, 4)
        q, k, v = qkv[0], qkv[1], qkv[2]
        scores = jnp.einsum("bhqd,bhkd->bhqk", q, k) * (Dh ** -0.5)
        p = _softmax(scores, axis=-1)
        o = jnp.einsum("bhqk,bhkd->bhqd", p, v)
        return (lambda x, *d: x.transpose(*d))(o, 0, 2, 1, 3).reshape(B, S, D) @ wo

    def _B_ref(x, w1, b1, w2):
        h = jnp.einsum("bsd,df->bsf", x, w1) + b1
        sp = jnp.log1p(jnp.exp(-jnp.abs(h))) + jnp.where(h > 0, h, jnp.zeros_like(h))
        act = h * jnp.tanh(sp)
        return jnp.einsum("bsf,fd->bsd", act, w2)

    x = A_x
    x = x + _A_ref(_layernorm(x, axis=-1), A_wqkv, A_wo)
    x = x + _B_ref(_layernorm(x, axis=-1), B_w1, B_b1, B_w2)
    x = x + _A_ref(_layernorm(x, axis=-1), A_wqkv, A_wo)
    x = x + _B_ref(_layernorm(x, axis=-1), B_w1, B_b1, B_w2)
    return x
```

```python
import functools
import math

import jax
import jax.numpy as jnp
from jax import lax
import jax.experimental.pallas as pl
import jax.experimental.pallas.tpu as pltpu

S = 2048
D = 512
H = 32
DH = 16
F = 1792
EPS = 1e-5

CK = 128 - DH
NCH = -(-S // CK)
LAST = S - (NCH - 1) * CK
TP = NCH * 128

M = 256
RB = 64
NQ = S // M
NQH = NQ // 2
T = NQH * H

RT = 256

QSCALE = (DH ** -0.5) * math.log2(math.e)
NEG = -1e30


def _ln(x):
    m = jnp.mean(x, axis=-1, keepdims=True)
    xc = x - m
    v = jnp.mean(xc * xc, axis=-1, keepdims=True)
    return xc * lax.rsqrt(v + EPS)


def _mish(h):
    u = jnp.exp(-jnp.abs(h))
    u2 = u * u
    pos = h >= 0
    n = jnp.where(pos, 1.0, u2) + 2.0 * u
    d = n + 2.0 * jnp.where(pos, u2, 1.0)
    return h * (n / d)


def _kernel(x_ref, wq_ref, wkt_ref, wv_ref, wo_ref, w1_ref, b1_ref, w2_ref,
            out_ref,
            xres, xn, xnp, q_s, kt_s, v_s, wt_s, o_s,
            s_a, s_b, l_a, l_b, li_a, li_b):
    f32 = jnp.float32
    bf16 = jnp.bfloat16

    xres[...] = x_ref[...].astype(f32)
    xnp[...] = jnp.zeros(xnp.shape, bf16)

    lane_rb = lax.broadcasted_iota(jnp.int32, (RB, 128), 1)

    def q_tile(t, chain, r0):
        h = t % H
        row = pl.multiple_of((chain * NQH + t // H) * M + r0, RB)
        qt = q_s[h // 8, pl.ds(row, RB), :]
        return pltpu.roll(qt, (128 - (h % 8) * DH) % 128, 1)

    def mxu_stage(t, s_ref, l_ref):
        h = t % H
        for j in range(NCH):
            s_ref[j] = jnp.dot(l_ref[j], wt_s[h, j], preferred_element_type=f32)

    def vpu_stage(t, chain, s_ref, l_ref, li_ref, first, last):
        for rb in range(M // RB):
            r0 = rb * RB
            rows = pl.ds(r0, RB)
            s0 = s_ref[0, rows, :]
            m = s0
            acc = s0
            for j in range(1, NCH - 1):
                sj = s_ref[j, rows, :]
                m = jnp.maximum(m, sj)
                acc = acc + sj
            sl = s_ref[NCH - 1, rows, :]
            acc = acc + sl
            if not first:
                tp = t - 1
                hp = tp % H
                orow = pl.multiple_of((chain * NQH + tp // H) * M + r0, RB)
                o = acc * li_ref[rows, :]
                o = pltpu.roll(o, (hp % 8) * DH, 1)
                old = o_s[hp // 8, pl.ds(orow, RB), :]
                o_s[hp // 8, pl.ds(orow, RB), :] = jnp.where(
                    lane_rb // DH == hp % 8, o, old)
            if last:
                continue
            m = jnp.maximum(m, jnp.where(lane_rb < DH + LAST, sl, NEG))
            m = jnp.where(lane_rb >= DH, m, NEG)
            mrow = jnp.max(m, axis=1, keepdims=True)
            qn = q_tile(jnp.minimum(t + 1, T - 1), chain, r0)
            ls = jnp.zeros((RB, 128), f32)
            for j in range(NCH):
                p = jnp.exp2(s_ref[j, rows, :] - mrow)
                if j == NCH - 1:
                    p = jnp.where(lane_rb < DH + LAST, p, 0.0)
                ls = ls + p
                l_ref[j, rows, :] = jnp.where(lane_rb < DH, qn, p).astype(bf16)
            lsum = jnp.sum(jnp.where(lane_rb >= DH, ls, 0.0), axis=1, keepdims=True)
            li_ref[rows, :] = jnp.broadcast_to(1.0 / lsum, (RB, 128))

    def init_l(chain, l_ref):
        for rb in range(M // RB):
            r0 = rb * RB
            rows = pl.ds(r0, RB)
            qn = q_tile(0, chain, r0)
            v = jnp.where(lane_rb < DH, qn, 0.0).astype(bf16)
            for j in range(NCH):
                l_ref[j, rows, :] = v

    def layer(_, carry):
        def ln1(i, c):
            r = pl.multiple_of(i * RT, RT)
            xn[pl.ds(r, RT), :] = _ln(xres[pl.ds(r, RT), :]).astype(bf16)
            return c
        lax.fori_loop(0, S // RT, ln1, 0)

        for j in range(NCH):
            n = CK if j < NCH - 1 else LAST
            xnp[j * 128 + DH:j * 128 + DH + n, :] = xn[j * CK:j * CK + n, :]

        def qproj(i, c):
            r = pl.multiple_of(i * RT, RT)
            q = jnp.dot(xn[pl.ds(r, RT), :], wq_ref[...],
                        preferred_element_type=f32) * QSCALE
            for g in range(4):
                q_s[g, pl.ds(r, RT), :] = q[:, g * 128:(g + 1) * 128]
            return c
        lax.fori_loop(0, S // RT, qproj, 0)

        def kvproj(j, c):
            r = pl.multiple_of(j * 128, 128)
            xc = xnp[pl.ds(r, 128), :]
            kt_s[j] = lax.dot_general(
                wkt_ref[...], xc, (((1,), (1,)), ((), ())),
                preferred_element_type=f32).astype(bf16)
            v = jnp.dot(xc, wv_ref[...], preferred_element_type=f32)
            for g in range(4):
                v_s[g, pl.ds(r, 128), :] = v[:, g * 128:(g + 1) * 128]
            return c
        lax.fori_loop(0, NCH, kvproj, 0)

        lane_w = lax.broadcasted_iota(jnp.int32, (CK, 128), 1)

        def wbuild(h, c):
            hp = (h + H - 1) % H
            kr = pl.multiple_of(h * DH, DH)
            for j in range(NCH):
                wt_s[h, j, 0:DH, :] = kt_s[j, pl.ds(kr, DH), :]
                v = v_s[hp // 8, j * 128 + DH:(j + 1) * 128, :]
                v = pltpu.roll(v, (128 - (hp % 8) * DH) % 128, 1)
                wt_s[h, j, DH:128, :] = jnp.where(lane_w < DH, v, 0.0).astype(bf16)
            return c
        lax.fori_loop(0, H, wbuild, 0)

        o_s[...] = jnp.zeros(o_s.shape, f32)

        init_l(0, l_a)
        init_l(1, l_b)
        mxu_stage(0, s_a, l_a)
        mxu_stage(0, s_b, l_b)
        vpu_stage(0, 0, s_a, l_a, li_a, True, False)

        def att(i, c):
            mxu_stage(i, s_a, l_a)
            vpu_stage(i - 1, 1, s_b, l_b, li_b, False, False)
            mxu_stage(i, s_b, l_b)
            vpu_stage(i, 0, s_a, l_a, li_a, False, False)
            return c
        mxu_stage(1, s_a, l_a)
        vpu_stage(0, 1, s_b, l_b, li_b, True, False)
        mxu_stage(1, s_b, l_b)
        vpu_stage(1, 0, s_a, l_a, li_a, False, False)
        lax.fori_loop(2, T, att, 0)
        mxu_stage(T, s_a, l_a)
        vpu_stage(T - 1, 1, s_b, l_b, li_b, False, False)
        mxu_stage(T, s_b, l_b)
        vpu_stage(T, 0, s_a, l_a, li_a, False, True)
        vpu_stage(T, 1, s_b, l_b, li_b, False, True)

        def ffn(i, c):
            r = pl.multiple_of(i * RT, RT)
            rows = pl.ds(r, RT)
            o = jnp.concatenate([o_s[g, rows, :] for g in range(4)], axis=1).astype(bf16)
            x1 = xres[rows, :] + jnp.dot(o, wo_ref[...], preferred_element_type=f32)
            xn2 = _ln(x1).astype(bf16)
            hh = jnp.dot(xn2, w1_ref[...], preferred_element_type=f32) + b1_ref[...].astype(f32)
            act = _mish(hh).astype(bf16)
            xres[rows, :] = x1 + jnp.dot(act, w2_ref[...], preferred_element_type=f32)
            return c
        lax.fori_loop(0, S // RT, ffn, 0)
        return carry

    lax.fori_loop(0, 2, layer, 0)
    out_ref[...] = xres[...].astype(out_ref.dtype)


@jax.jit
def pallas_interleave_layers__mha_block__dense_activation_mish__prompt_kernel(
    A_x: jax.Array,
    A_wqkv: jax.Array,
    A_wo: jax.Array,
    B_x: jax.Array,
    B_w1: jax.Array,
    B_b1: jax.Array,
    B_w2: jax.Array,
):
    x = A_x.reshape(S, D)
    wq = A_wqkv[:, :D]
    wkt = A_wqkv[:, D:2 * D].T
    wv = A_wqkv[:, 2 * D:]
    b1 = B_b1.reshape(1, F)

    f32 = jnp.float32
    bf16 = jnp.bfloat16
    scratch = [
        pltpu.VMEM((S, D), f32),
        pltpu.VMEM((S, D), bf16),
        pltpu.VMEM((TP, D), bf16),
        pltpu.VMEM((4, S, 128), f32),
        pltpu.VMEM((NCH, D, 128), bf16),
        pltpu.VMEM((4, TP, 128), f32),
        pltpu.VMEM((H, NCH, 128, 128), bf16),
        pltpu.VMEM((4, S, 128), f32),
        pltpu.VMEM((NCH, M, 128), f32),
        pltpu.VMEM((NCH, M, 128), f32),
        pltpu.VMEM((NCH, M, 128), bf16),
        pltpu.VMEM((NCH, M, 128), bf16),
        pltpu.VMEM((M, 128), f32),
        pltpu.VMEM((M, 128), f32),
    ]
    out = pl.pallas_call(
        _kernel,
        out_shape=jax.ShapeDtypeStruct((S, D), A_x.dtype),
        scratch_shapes=scratch,
        compiler_params=pltpu.CompilerParams(vmem_limit_bytes=100 * 1024 * 1024),
    )(x, wq, wkt, wv, A_wo, B_w1, b1, B_w2)
    return out.reshape(A_x.shape)
```

```python
import functools
import math

import jax
import jax.numpy as jnp
from jax import lax
import jax.experimental.pallas as pl
import jax.experimental.pallas.tpu as pltpu

S = 2048
D = 512
H = 32
DH = 16
F = 1792
EPS = 1e-5

K0 = DH + 1
CK = 128 - K0
NCH = -(-S // CK)
LAST = S - (NCH - 1) * CK
TP = NCH * 128

M = 512
RB = 64
NQ = S // M
NQH = NQ // 2
T = NQH * H

RT = 256

QSCALE = (DH ** -0.5) * math.log2(math.e)
NEG = -1e30


def _ln(x):
    m = jnp.mean(x, axis=-1, keepdims=True)
    xc = x - m
    v = jnp.mean(xc * xc, axis=-1, keepdims=True)
    return xc * lax.rsqrt(v + EPS)


def _mish(h):
    u = jnp.exp(-jnp.abs(h))
    u2 = u * u
    pos = h >= 0
    n = jnp.where(pos, 1.0, u2) + 2.0 * u
    d = n + 2.0 * jnp.where(pos, u2, 1.0)
    return h * (n / d)


def _kernel(x_hbm, wqkv_hbm, wo_hbm, w1_hbm, b1_hbm, w2_hbm,
            out_hbm,
            x_ref, wqkv_ref, wo_ref, w1_ref, b1_ref, w2_ref, in_sems, out_sems,
            wkt_ref, xres, xn, xnp, q_s, wt_s, o_s,
            s_a, s_b, m_a, m_b):
    f32 = jnp.float32
    bf16 = jnp.bfloat16
    u32 = jnp.uint32

    def pk(x):
        return pltpu.bitcast(x, u32)

    def upk(x):
        return pltpu.bitcast(x, bf16)

    wt_u = wt_s.bitcast(u32)
    in_copies = [
        pltpu.make_async_copy(src, dst, in_sems.at[i])
        for i, (src, dst) in enumerate([
            (x_hbm.at[0], x_ref), (wqkv_hbm, wqkv_ref), (wo_hbm, wo_ref),
            (w1_hbm, w1_ref), (b1_hbm, b1_ref), (w2_hbm, w2_ref)])]
    for cp in in_copies:
        cp.start()

    def out_copy(i):
        rows = pl.ds(pl.multiple_of(i * RT, RT), RT)
        return pltpu.make_async_copy(x_ref.at[rows, :], out_hbm.at[0, rows, :], out_sems.at[i])

    in_copies[0].wait()
    xres[...] = x_ref[...].astype(f32)
    in_copies[1].wait()
    wkt_ref[...] = wqkv_ref[:, D:2 * D].astype(f32).T.astype(bf16)
    xnp[...] = jnp.zeros(xnp.shape, bf16)

    lane_rb = lax.broadcasted_iota(jnp.int32, (RB, 128), 1)
    lane_h = lax.broadcasted_iota(jnp.int32, (RB // 2, 128), 1)

    lane_m = lax.broadcasted_iota(jnp.int32, (M, 128), 1)

    def q_tile(t, chain):
        h = t % H
        row = pl.multiple_of((chain * NQH + t // H) * M, M)
        qt = q_s[h // 8, pl.ds(row, M), :]
        return pltpu.roll(qt, (128 - (h % 8) * DH) % 128, 1)

    def cm_stage(t, chain, s_ref, m_ref, first=False):
        h = t % H
        qn = q_tile(jnp.minimum(t, T - 1), chain)
        for j in range(NCH):
            if first:
                p = 0.0
            else:
                p = jnp.exp2(s_ref[j] - m_ref[...])
                if j == NCH - 1:
                    p = jnp.where(lane_m < K0 + LAST, p, 0.0)
            lhs = jnp.where(lane_m < K0, qn, p).astype(bf16)
            s_ref[j] = jnp.dot(lhs, upk(wt_u[h, j]), preferred_element_type=f32)

    def b_stage(t, chain, s_ref, m_ref, first=False, last=False):
        for rb in range(M // RB):
            r0 = rb * RB
            rows = pl.ds(r0, RB)
            s0 = s_ref[0, rows, :]
            m = s0
            acc = s0
            for j in range(1, NCH - 1):
                sj = s_ref[j, rows, :]
                m = jnp.maximum(m, sj)
                acc = acc + sj
            sl = s_ref[NCH - 1, rows, :]
            acc = acc + sl
            if not first:
                tp = t - 1
                hp = tp % H
                orow = pl.multiple_of((chain * NQH + tp // H) * M + r0, RB)
                o = acc / acc[:, DH:DH + 1]
                o = pltpu.roll(o, (hp % 8) * DH, 1)
                old = o_s[hp // 8, pl.ds(orow, RB), :]
                o_s[hp // 8, pl.ds(orow, RB), :] = jnp.where(
                    lane_rb // DH == hp % 8, o, old)
            if last:
                continue
            m = jnp.maximum(m, jnp.where(lane_rb < K0 + LAST, sl, NEG))
            m = jnp.where(lane_rb >= K0, m, NEG)
            mrow = jnp.max(m, axis=1, keepdims=True)
            m_ref[rows, :] = jnp.broadcast_to(mrow, (RB, 128))

    def layer(li, carry):
        def ln1(i, c):
            r = pl.multiple_of(i * RT, RT)
            xn[pl.ds(r, RT), :] = _ln(xres[pl.ds(r, RT), :]).astype(bf16)
            return c
        with jax.named_scope('ln1'):
            lax.fori_loop(0, S // RT, ln1, 0)

        with jax.named_scope('xnp'):
            for j in range(NCH):
                n = CK if j < NCH - 1 else LAST
                xnp[j * 128 + K0:j * 128 + K0 + n, :] = xn[j * CK:j * CK + n, :]

        def qproj(i, c):
            r = pl.multiple_of(i * RT, RT)
            q = jnp.dot(xn[pl.ds(r, RT), :], wqkv_ref[:, 0:D],
                        preferred_element_type=f32) * QSCALE
            for g in range(4):
                q_s[g, pl.ds(r, RT), :] = q[:, g * 128:(g + 1) * 128]
            return c
        with jax.named_scope('qproj'):
            lax.fori_loop(0, S // RT, qproj, 0)

        lane_w = lax.broadcasted_iota(jnp.int32, (128 - DH, 128), 1)
        row_w = lax.broadcasted_iota(jnp.int32, (128 - DH, 128), 0) + DH

        def kvproj(j, c):
            r = pl.multiple_of(j * 128, 128)
            xc = xnp[pl.ds(r, 128), :]
            v = jnp.dot(xc, wqkv_ref[:, 2 * D:3 * D], preferred_element_type=f32)
            kt = lax.dot_general(
                wkt_ref[...], xc, (((1,), (1,)), ((), ())),
                preferred_element_type=f32).astype(bf16)
            nvalid = jnp.where(j < NCH - 1, CK, LAST)
            ones = jnp.where((lane_w == DH) & (row_w >= K0) & (row_w < K0 + nvalid), 1.0, 0.0)
            for h in range(H):
                wt_s[h, j, 0:DH, :] = kt[h * DH:(h + 1) * DH, :]
                vt = v[DH:, (h // 8) * 128:(h // 8 + 1) * 128]
                if h % 8:
                    vt = pltpu.roll(vt, 128 - (h % 8) * DH, 1)
                wt_s[(h + 1) % H, j, DH:128, :] = jnp.where(lane_w < DH, vt, ones).astype(bf16)
            return c
        with jax.named_scope('kvproj'):
            lax.fori_loop(0, NCH, kvproj, 0)

        o_s[...] = jnp.zeros(o_s.shape, f32)

        cm_stage(0, 0, s_a, m_a, first=True)
        cm_stage(0, 1, s_b, m_b, first=True)
        b_stage(0, 0, s_a, m_a, first=True)
        cm_stage(1, 0, s_a, m_a)
        b_stage(0, 1, s_b, m_b, first=True)
        cm_stage(1, 1, s_b, m_b)
        b_stage(1, 0, s_a, m_a)

        def att(i, c):
            cm_stage(i, 0, s_a, m_a)
            b_stage(i - 1, 1, s_b, m_b)
            cm_stage(i, 1, s_b, m_b)
            b_stage(i, 0, s_a, m_a)
            return c
        with jax.named_scope('att'):
            lax.fori_loop(2, T, att, 0)
        cm_stage(T, 0, s_a, m_a)
        b_stage(T - 1, 1, s_b, m_b)
        cm_stage(T, 1, s_b, m_b)
        b_stage(T, 0, s_a, m_a, last=True)
        b_stage(T, 1, s_b, m_b, last=True)

        @pl.when(li == 0)
        def _():
            for cp in in_copies[2:]:
                cp.wait()

        def ffn(i, c):
            r = pl.multiple_of(i * RT, RT)
            rows = pl.ds(r, RT)
            o = jnp.concatenate([o_s[g, rows, :] for g in range(4)], axis=1).astype(bf16)
            x1 = xres[rows, :] + jnp.dot(o, wo_ref[...], preferred_element_type=f32)
            xn2 = _ln(x1).astype(bf16)
            hh = jnp.dot(xn2, w1_ref[...], preferred_element_type=f32) + b1_ref[...].astype(f32)[None, :]
            act = _mish(hh).astype(bf16)
            x2 = x1 + jnp.dot(act, w2_ref[...], preferred_element_type=f32)
            xres[rows, :] = x2

            @pl.when(li == 1)
            def _():
                x_ref[rows, :] = x2.astype(bf16)
                out_copy(i).start()
            return c
        with jax.named_scope('ffn'):
            lax.fori_loop(0, S // RT, ffn, 0)
        return carry

    lax.fori_loop(0, 2, layer, 0)
    for i in range(S // RT):
        out_copy(i).wait()


@jax.jit
def pallas_interleave_layers__mha_block__dense_activation_mish__prompt_kernel(
    A_x: jax.Array,
    A_wqkv: jax.Array,
    A_wo: jax.Array,
    B_x: jax.Array,
    B_w1: jax.Array,
    B_b1: jax.Array,
    B_w2: jax.Array,
):
    f32 = jnp.float32
    bf16 = jnp.bfloat16
    u32 = jnp.uint32
    scratch = [
        pltpu.VMEM((S, D), bf16),
        pltpu.VMEM((D, 3 * D), bf16),
        pltpu.VMEM((D, D), bf16),
        pltpu.VMEM((D, F), bf16),
        pltpu.VMEM((F,), bf16),
        pltpu.VMEM((F, D), bf16),
        pltpu.SemaphoreType.DMA((6,)),
        pltpu.SemaphoreType.DMA((S // RT,)),
        pltpu.VMEM((D, D), bf16),
        pltpu.VMEM((S, D), f32),
        pltpu.VMEM((S, D), bf16),
        pltpu.VMEM((TP, D), bf16),
        pltpu.VMEM((4, S, 128), f32),
        pltpu.VMEM((H, NCH, 128, 128), bf16),
        pltpu.VMEM((4, S, 128), f32),
        pltpu.VMEM((NCH, M, 128), f32),
        pltpu.VMEM((NCH, M, 128), f32),
        pltpu.VMEM((M, 128), f32),
        pltpu.VMEM((M, 128), f32),
    ]
    out = pl.pallas_call(
        _kernel,
        out_shape=jax.ShapeDtypeStruct(A_x.shape, A_x.dtype),
        in_specs=[pl.BlockSpec(memory_space=pl.ANY)] * 6,
        out_specs=pl.BlockSpec(memory_space=pl.ANY),
        scratch_shapes=scratch,
        compiler_params=pltpu.CompilerParams(vmem_limit_bytes=100 * 1024 * 1024),
    )(A_x, A_wqkv, A_wo, B_w1, B_b1, B_w2)
    return out
```

```python
import math

import jax
import jax.numpy as jnp
from jax import lax
import jax.experimental.pallas as pl
import jax.experimental.pallas.tpu as pltpu

S = 2048
D = 512
H = 32
DH = 16
F = 1792
EPS = 1e-5

K0 = DH + 1
CK = 128 - K0
NCH = -(-S // CK)
LAST = S - (NCH - 1) * CK
TP = NCH * 128

M = 1024
RB = 64
NQ = S // M
NQH = NQ // 2
T = NQH * H

RT = 512

QSCALE = (DH ** -0.5) * math.log2(math.e)
NEG = -1e30


def _ln(x):
    m = jnp.mean(x, axis=-1, keepdims=True)
    xc = x - m
    v = jnp.mean(xc * xc, axis=-1, keepdims=True)
    return xc * lax.rsqrt(v + EPS)


def _mish(h):
    u = jnp.exp(-jnp.abs(h))
    u2 = u * u
    pos = h >= 0
    n = jnp.where(pos, 1.0, u2) + 2.0 * u
    d = n + 2.0 * jnp.where(pos, u2, 1.0)
    return h * (n / d)


def _kernel(x_hbm, wqkv_hbm, wo_hbm, w1_hbm, b1_hbm, w2_hbm,
            out_hbm,
            x_ref, wqkv_ref, wo_ref, w1_ref, b1_ref, w2_ref, in_sems, out_sems,
            wkt_ref, xres, xn, xnp, q_s, wt_s, o_s,
            s_a, s_b, m_a, m_b, qn_s):
    f32 = jnp.float32
    bf16 = jnp.bfloat16
    u32 = jnp.uint32

    def upk(x):
        return pltpu.bitcast(x, bf16)

    wt_u = wt_s.bitcast(u32)
    in_copies = [
        pltpu.make_async_copy(src, dst, in_sems.at[i])
        for i, (src, dst) in enumerate([
            (x_hbm.at[0], x_ref), (wqkv_hbm, wqkv_ref), (wo_hbm, wo_ref),
            (w1_hbm, w1_ref), (b1_hbm, b1_ref), (w2_hbm, w2_ref)])]
    for cp in in_copies:
        cp.start()

    def out_copy(i):
        rows = pl.ds(pl.multiple_of(i * RT, RT), RT)
        return pltpu.make_async_copy(x_ref.at[rows, :], out_hbm.at[0, rows, :], out_sems.at[i])

    xnp[...] = jnp.zeros(xnp.shape, bf16)
    in_copies[0].wait()

    def ln0(i, c):
        rows = pl.ds(pl.multiple_of(i * 256, 256), 256)
        xt = x_ref[rows, :].astype(f32)
        xres[rows, :] = xt
        xn[rows, :] = _ln(xt).astype(bf16)
        return c
    lax.fori_loop(0, S // 256, ln0, 0)
    in_copies[1].wait()
    wkt_ref[...] = wqkv_ref[:, D:2 * D].astype(f32).T.astype(bf16)

    lane_rb = lax.broadcasted_iota(jnp.int32, (RB, 128), 1)
    lane_m = lax.broadcasted_iota(jnp.int32, (M, 128), 1)

    def q_tile(t, chain, r0):
        h = t % H
        row = pl.multiple_of((chain * NQH + t // H) * M + r0, RB)
        qt = q_s[h // 8, pl.ds(row, RB), :]
        return pltpu.roll(qt, (128 - (h % 8) * DH) % 128, 1)

    def cm_stage(t, chain, s_ref, m_ref, first=False):
        h = t % H
        if first:
            for rb in range(M // RB):
                qn_s[chain, pl.ds(rb * RB, RB), :] = q_tile(0, chain, rb * RB)
        qn = qn_s[chain]
        for j in range(NCH):
            if first:
                p = 0.0
            else:
                p = jnp.exp2(s_ref[j] - m_ref[...])
                if j == NCH - 1:
                    p = jnp.where(lane_m < K0 + LAST, p, 0.0)
            lhs = jnp.where(lane_m < K0, qn, p).astype(bf16)
            s_ref[j] = jnp.dot(lhs, upk(wt_u[h, j]), preferred_element_type=f32)

    def b_stage(t, chain, s_ref, m_ref, first=False, last=False):
        for rb in range(M // RB):
            r0 = rb * RB
            rows = pl.ds(r0, RB)
            s0 = s_ref[0, rows, :]
            m = s0
            acc = s0
            for j in range(1, NCH - 1):
                sj = s_ref[j, rows, :]
                m = jnp.maximum(m, sj)
                acc = acc + sj
            sl = s_ref[NCH - 1, rows, :]
            acc = acc + sl
            if not first:
                tp = t - 1
                hp = tp % H
                orow = pl.multiple_of((chain * NQH + tp // H) * M + r0, RB)
                o = acc / acc[:, DH:DH + 1]
                o = pltpu.roll(o, (hp % 8) * DH, 1)
                old = o_s[hp // 8, pl.ds(orow, RB), :]
                o_s[hp // 8, pl.ds(orow, RB), :] = jnp.where(
                    lane_rb // DH == hp % 8, o, old)
            if last:
                continue
            m = jnp.maximum(m, jnp.where(lane_rb < K0 + LAST, sl, NEG))
            m = jnp.where(lane_rb >= K0, m, NEG)
            mrow = jnp.max(m, axis=1, keepdims=True)
            m_ref[rows, :] = jnp.broadcast_to(mrow, (RB, 128))
            qn_s[chain, rows, :] = q_tile(jnp.minimum(t + 1, T - 1), chain, r0)

    def layer(li, carry):
        def qproj(i, c):
            r = pl.multiple_of(i * RT, RT)
            q = jnp.dot(xn[pl.ds(r, RT), :], wqkv_ref[:, 0:D],
                        preferred_element_type=f32) * QSCALE
            for g in range(4):
                q_s[g, pl.ds(r, RT), :] = q[:, g * 128:(g + 1) * 128]
            return c
        lax.fori_loop(0, S // RT, qproj, 0)

        for j in range(NCH):
            n = CK if j < NCH - 1 else LAST
            xnp[j * 128 + K0:j * 128 + K0 + n, :] = xn[j * CK:j * CK + n, :]

        lane_w = lax.broadcasted_iota(jnp.int32, (128 - DH, 128), 1)
        row_w = lax.broadcasted_iota(jnp.int32, (128 - DH, 128), 0) + DH

        def kvproj(j, c):
            r = pl.multiple_of(j * 128, 128)
            xc = xnp[pl.ds(r, 128), :]
            v = jnp.dot(xc, wqkv_ref[:, 2 * D:3 * D], preferred_element_type=f32)
            kt = lax.dot_general(
                wkt_ref[...], xc, (((1,), (1,)), ((), ())),
                preferred_element_type=f32).astype(bf16)
            nvalid = jnp.where(j < NCH - 1, CK, LAST)
            ones = jnp.where((lane_w == DH) & (row_w >= K0) & (row_w < K0 + nvalid), 1.0, 0.0)
            for h in range(H):
                wt_s[h, j, 0:DH, :] = kt[h * DH:(h + 1) * DH, :]
                vt = v[DH:, (h // 8) * 128:(h // 8 + 1) * 128]
                if h % 8:
                    vt = pltpu.roll(vt, 128 - (h % 8) * DH, 1)
                wt_s[(h + 1) % H, j, DH:128, :] = jnp.where(lane_w < DH, vt, ones).astype(bf16)
            return c
        lax.fori_loop(0, NCH, kvproj, 0, unroll=2)

        o_s[...] = jnp.zeros(o_s.shape, f32)

        cm_stage(0, 0, s_a, m_a, first=True)
        cm_stage(0, 1, s_b, m_b, first=True)
        b_stage(0, 0, s_a, m_a, first=True)
        cm_stage(1, 0, s_a, m_a)
        b_stage(0, 1, s_b, m_b, first=True)
        cm_stage(1, 1, s_b, m_b)
        b_stage(1, 0, s_a, m_a)

        def att(i, c):
            cm_stage(i, 0, s_a, m_a)
            b_stage(i - 1, 1, s_b, m_b)
            cm_stage(i, 1, s_b, m_b)
            b_stage(i, 0, s_a, m_a)
            return c
        lax.fori_loop(2, T, att, 0)
        cm_stage(T, 0, s_a, m_a)
        b_stage(T - 1, 1, s_b, m_b)
        cm_stage(T, 1, s_b, m_b)
        b_stage(T, 0, s_a, m_a, last=True)
        b_stage(T, 1, s_b, m_b, last=True)

        @pl.when(li == 0)
        def _():
            for cp in in_copies[2:]:
                cp.wait()

        def ffn(i, c):
            r = pl.multiple_of(i * RT, RT)
            rows = pl.ds(r, RT)
            o = jnp.concatenate([o_s[g, rows, :] for g in range(4)], axis=1).astype(bf16)
            x1 = xres[rows, :] + jnp.dot(o, wo_ref[...], preferred_element_type=f32)
            xn2 = _ln(x1).astype(bf16)
            hh = jnp.dot(xn2, w1_ref[...], preferred_element_type=f32) + b1_ref[...].astype(f32)[None, :]
            act = _mish(hh).astype(bf16)
            x2 = x1 + jnp.dot(act, w2_ref[...], preferred_element_type=f32)
            xres[rows, :] = x2
            xn[rows, :] = _ln(x2).astype(bf16)

            @pl.when(li == 1)
            def _():
                x_ref[rows, :] = x2.astype(bf16)
                out_copy(i).start()
            return c
        lax.fori_loop(0, S // RT, ffn, 0)
        return carry

    lax.fori_loop(0, 2, layer, 0)
    for i in range(S // RT):
        out_copy(i).wait()


@jax.jit
def pallas_interleave_layers__mha_block__dense_activation_mish__prompt_kernel(
    A_x: jax.Array,
    A_wqkv: jax.Array,
    A_wo: jax.Array,
    B_x: jax.Array,
    B_w1: jax.Array,
    B_b1: jax.Array,
    B_w2: jax.Array,
):
    f32 = jnp.float32
    bf16 = jnp.bfloat16
    scratch = [
        pltpu.VMEM((S, D), bf16),
        pltpu.VMEM((D, 3 * D), bf16),
        pltpu.VMEM((D, D), bf16),
        pltpu.VMEM((D, F), bf16),
        pltpu.VMEM((F,), bf16),
        pltpu.VMEM((F, D), bf16),
        pltpu.SemaphoreType.DMA((6,)),
        pltpu.SemaphoreType.DMA((S // RT,)),
        pltpu.VMEM((D, D), bf16),
        pltpu.VMEM((S, D), f32),
        pltpu.VMEM((S, D), bf16),
        pltpu.VMEM((TP, D), bf16),
        pltpu.VMEM((4, S, 128), f32),
        pltpu.VMEM((H, NCH, 128, 128), bf16),
        pltpu.VMEM((4, S, 128), f32),
        pltpu.VMEM((NCH, M, 128), f32),
        pltpu.VMEM((NCH, M, 128), f32),
        pltpu.VMEM((M, 128), f32),
        pltpu.VMEM((M, 128), f32),
        pltpu.VMEM((2, M, 128), f32),
    ]
    out = pl.pallas_call(
        _kernel,
        out_shape=jax.ShapeDtypeStruct(A_x.shape, A_x.dtype),
        in_specs=[pl.BlockSpec(memory_space=pl.ANY)] * 6,
        out_specs=pl.BlockSpec(memory_space=pl.ANY),
        scratch_shapes=scratch,
        compiler_params=pltpu.CompilerParams(vmem_limit_bytes=100 * 1024 * 1024),
    )(A_x, A_wqkv, A_wo, B_w1, B_b1, B_w2)
    return out
```

```python
import math

import jax
import jax.numpy as jnp
from jax import lax
import jax.experimental.pallas as pl
import jax.experimental.pallas.tpu as pltpu

S = 2048
D = 512
H = 32
DH = 16
F = 1792
EPS = 1e-5

K0 = DH + 1
CK = 128 - K0
NCH = -(-S // CK)
LAST = S - (NCH - 1) * CK
TP = NCH * 128

M = 1024
RB = 64
NQ = S // M
NQH = NQ // 2
T = NQH * H

RT = 512

QSCALE = (DH ** -0.5) * math.log2(math.e)
NEG = -1e30


def _ln(x):
    m = jnp.mean(x, axis=-1, keepdims=True)
    xc = x - m
    v = jnp.mean(xc * xc, axis=-1, keepdims=True)
    return xc * lax.rsqrt(v + EPS)


def _mish(h):
    u = jnp.exp(-jnp.abs(h))
    u2 = u * u
    pos = h >= 0
    n = jnp.where(pos, 1.0, u2) + 2.0 * u
    d = n + 2.0 * jnp.where(pos, u2, 1.0)
    return h * (n / d)


def _kernel(x_hbm, wqkv_hbm, wo_hbm, w1_hbm, b1_hbm, w2_hbm,
            out_hbm,
            x_ref, wqkv_ref, wo_ref, w1_ref, b1_ref, w2_ref, x_sems, in_sems, out_sems,
            wkt_ref, xres, xn, xnp, q_s, wt_s, o_s,
            s_a, s_b, m_a, m_b, qn_s):
    f32 = jnp.float32
    bf16 = jnp.bfloat16
    u32 = jnp.uint32

    def upk(x):
        return pltpu.bitcast(x, bf16)

    wt_u = wt_s.bitcast(u32)
    NXC = 8
    XR = S // NXC

    def x_copy(i):
        rows = pl.ds(pl.multiple_of(i * XR, XR), XR)
        return pltpu.make_async_copy(x_hbm.at[0, rows, :], x_ref.at[rows, :], x_sems.at[i])

    in_copies = [
        pltpu.make_async_copy(src, dst, in_sems.at[i])
        for i, (src, dst) in enumerate([
            (wqkv_hbm, wqkv_ref), (wo_hbm, wo_ref),
            (w1_hbm, w1_ref), (b1_hbm, b1_ref), (w2_hbm, w2_ref)])]
    for i in range(NXC):
        x_copy(i).start()
    in_copies[0].start()

    def out_copy(i):
        rows = pl.ds(pl.multiple_of(i * RT, RT), RT)
        return pltpu.make_async_copy(x_ref.at[rows, :], out_hbm.at[0, rows, :], out_sems.at[i])

    xnp[...] = jnp.zeros(xnp.shape, bf16)

    def ln0(i, c):
        x_copy(i).wait()
        rows = pl.ds(pl.multiple_of(i * XR, XR), XR)
        xt = x_ref[rows, :].astype(f32)
        xres[rows, :] = xt
        xn[rows, :] = _ln(xt).astype(bf16)
        return c
    lax.fori_loop(0, NXC, ln0, 0)
    in_copies[0].wait()
    for cp in in_copies[1:]:
        cp.start()
    wkt_ref[...] = wqkv_ref[:, D:2 * D].astype(f32).T.astype(bf16)

    lane_rb = lax.broadcasted_iota(jnp.int32, (RB, 128), 1)
    lane_m = lax.broadcasted_iota(jnp.int32, (M, 128), 1)

    def q_tile(t, chain, r0):
        h = t % H
        row = pl.multiple_of((chain * NQH + t // H) * M + r0, RB)
        qt = q_s[h // 8, pl.ds(row, RB), :]
        return pltpu.roll(qt, (128 - (h % 8) * DH) % 128, 1)

    def cm_stage(t, chain, s_ref, m_ref, first=False):
        h = t % H
        if first:
            for rb in range(M // RB):
                qn_s[chain, pl.ds(rb * RB, RB), :] = q_tile(0, chain, rb * RB)
        qn = qn_s[chain]
        for j in range(NCH):
            if first:
                p = 0.0
            else:
                p = jnp.exp2(s_ref[j] - m_ref[...])
                if j == NCH - 1:
                    p = jnp.where(lane_m < K0 + LAST, p, 0.0)
            lhs = jnp.where(lane_m < K0, qn, p).astype(bf16)
            s_ref[j] = jnp.dot(lhs, upk(wt_u[h, j]), preferred_element_type=f32)

    def b_stage(t, chain, s_ref, m_ref, first=False, last=False):
        for rb in range(M // RB):
            r0 = rb * RB
            rows = pl.ds(r0, RB)
            s0 = s_ref[0, rows, :]
            m = s0
            acc = s0
            for j in range(1, NCH - 1):
                sj = s_ref[j, rows, :]
                m = jnp.maximum(m, sj)
                acc = acc + sj
            sl = s_ref[NCH - 1, rows, :]
            acc = acc + sl
            if not first:
                tp = t - 1
                hp = tp % H
                orow = pl.multiple_of((chain * NQH + tp // H) * M + r0, RB)
                o = acc / acc[:, DH:DH + 1]
                o = pltpu.roll(o, (hp % 8) * DH, 1)
                old = o_s[hp // 8, pl.ds(orow, RB), :]
                o_s[hp // 8, pl.ds(orow, RB), :] = jnp.where(
                    lane_rb // DH == hp % 8, o, old)
            if last:
                continue
            m = jnp.maximum(m, jnp.where(lane_rb < K0 + LAST, sl, NEG))
            m = jnp.where(lane_rb >= K0, m, NEG)
            mrow = jnp.max(m, axis=1, keepdims=True)
            m_ref[rows, :] = jnp.broadcast_to(mrow, (RB, 128))
            qn_s[chain, rows, :] = q_tile(jnp.minimum(t + 1, T - 1), chain, r0)

    def layer(li, carry):
        def qproj(i, c):
            r = pl.multiple_of(i * RT, RT)
            q = jnp.dot(xn[pl.ds(r, RT), :], wqkv_ref[:, 0:D],
                        preferred_element_type=f32) * QSCALE
            for g in range(4):
                q_s[g, pl.ds(r, RT), :] = q[:, g * 128:(g + 1) * 128]
            return c
        lax.fori_loop(0, S // RT, qproj, 0)

        for j in range(NCH):
            n = CK if j < NCH - 1 else LAST
            xnp[j * 128 + K0:j * 128 + K0 + n, :] = xn[j * CK:j * CK + n, :]

        lane_w = lax.broadcasted_iota(jnp.int32, (128 - DH, 128), 1)
        row_w = lax.broadcasted_iota(jnp.int32, (128 - DH, 128), 0) + DH

        def kvproj(j, c):
            r = pl.multiple_of(j * 128, 128)
            xc = xnp[pl.ds(r, 128), :]
            v = jnp.dot(xc, wqkv_ref[:, 2 * D:3 * D], preferred_element_type=f32)
            kt = lax.dot_general(
                wkt_ref[...], xc, (((1,), (1,)), ((), ())),
                preferred_element_type=f32).astype(bf16)
            nvalid = jnp.where(j < NCH - 1, CK, LAST)
            ones = jnp.where((lane_w == DH) & (row_w >= K0) & (row_w < K0 + nvalid), 1.0, 0.0)
            for h in range(H):
                wt_s[h, j, 0:DH, :] = kt[h * DH:(h + 1) * DH, :]
                vt = v[DH:, (h // 8) * 128:(h // 8 + 1) * 128]
                if h % 8:
                    vt = pltpu.roll(vt, 128 - (h % 8) * DH, 1)
                wt_s[(h + 1) % H, j, DH:128, :] = jnp.where(lane_w < DH, vt, ones).astype(bf16)
            return c
        lax.fori_loop(0, NCH, kvproj, 0, unroll=2)

        o_s[...] = jnp.zeros(o_s.shape, f32)

        cm_stage(0, 0, s_a, m_a, first=True)
        cm_stage(0, 1, s_b, m_b, first=True)
        b_stage(0, 0, s_a, m_a, first=True)
        cm_stage(1, 0, s_a, m_a)
        b_stage(0, 1, s_b, m_b, first=True)
        cm_stage(1, 1, s_b, m_b)
        b_stage(1, 0, s_a, m_a)

        def att(i, c):
            cm_stage(i, 0, s_a, m_a)
            b_stage(i - 1, 1, s_b, m_b)
            cm_stage(i, 1, s_b, m_b)
            b_stage(i, 0, s_a, m_a)
            return c
        lax.fori_loop(2, T, att, 0)
        cm_stage(T, 0, s_a, m_a)
        b_stage(T - 1, 1, s_b, m_b)
        cm_stage(T, 1, s_b, m_b)
        b_stage(T, 0, s_a, m_a, last=True)
        b_stage(T, 1, s_b, m_b, last=True)

        @pl.when(li == 0)
        def _():
            for cp in in_copies[1:]:
                cp.wait()

        def ffn(i, c):
            r = pl.multiple_of(i * RT, RT)
            rows = pl.ds(r, RT)
            o = jnp.concatenate([o_s[g, rows, :] for g in range(4)], axis=1).astype(bf16)
            x1 = xres[rows, :] + jnp.dot(o, wo_ref[...], preferred_element_type=f32)
            xn2 = _ln(x1).astype(bf16)
            hh = jnp.dot(xn2, w1_ref[...], preferred_element_type=f32) + b1_ref[...].astype(f32)[None, :]
            act = _mish(hh).astype(bf16)
            x2 = x1 + jnp.dot(act, w2_ref[...], preferred_element_type=f32)
            xres[rows, :] = x2
            xn[rows, :] = _ln(x2).astype(bf16)

            @pl.when(li == 1)
            def _():
                x_ref[rows, :] = x2.astype(bf16)
                out_copy(i).start()
            return c
        lax.fori_loop(0, S // RT, ffn, 0)
        return carry

    lax.fori_loop(0, 2, layer, 0)
    for i in range(S // RT):
        out_copy(i).wait()


@jax.jit
def pallas_interleave_layers__mha_block__dense_activation_mish__prompt_kernel(
    A_x: jax.Array,
    A_wqkv: jax.Array,
    A_wo: jax.Array,
    B_x: jax.Array,
    B_w1: jax.Array,
    B_b1: jax.Array,
    B_w2: jax.Array,
):
    f32 = jnp.float32
    bf16 = jnp.bfloat16
    scratch = [
        pltpu.VMEM((S, D), bf16),
        pltpu.VMEM((D, 3 * D), bf16),
        pltpu.VMEM((D, D), bf16),
        pltpu.VMEM((D, F), bf16),
        pltpu.VMEM((F,), bf16),
        pltpu.VMEM((F, D), bf16),
        pltpu.SemaphoreType.DMA((8,)),
        pltpu.SemaphoreType.DMA((5,)),
        pltpu.SemaphoreType.DMA((S // RT,)),
        pltpu.VMEM((D, D), bf16),
        pltpu.VMEM((S, D), f32),
        pltpu.VMEM((S, D), bf16),
        pltpu.VMEM((TP, D), bf16),
        pltpu.VMEM((4, S, 128), f32),
        pltpu.VMEM((H, NCH, 128, 128), bf16),
        pltpu.VMEM((4, S, 128), f32),
        pltpu.VMEM((NCH, M, 128), f32),
        pltpu.VMEM((NCH, M, 128), f32),
        pltpu.VMEM((M, 128), f32),
        pltpu.VMEM((M, 128), f32),
        pltpu.VMEM((2, M, 128), f32),
    ]
    out = pl.pallas_call(
        _kernel,
        out_shape=jax.ShapeDtypeStruct(A_x.shape, A_x.dtype),
        in_specs=[pl.BlockSpec(memory_space=pl.ANY)] * 6,
        out_specs=pl.BlockSpec(memory_space=pl.ANY),
        scratch_shapes=scratch,
        compiler_params=pltpu.CompilerParams(vmem_limit_bytes=100 * 1024 * 1024),
    )(A_x, A_wqkv, A_wo, B_w1, B_b1, B_w2)
    return out
```
